```python
import os as _os
_os.environ.setdefault("JAX_PLATFORMS", "cpu")
import jax
import jax.numpy as jnp

def _softmax(x, axis=-1):
    return jax.nn.softmax(x, axis=axis)
def _gelu(x):
    return jax.nn.gelu(x, approximate=True)
def _silu(x):
    return jax.nn.silu(x)
def _sigmoid(x):
    return jax.nn.sigmoid(x)
def _layernorm(x, axis=-1, eps=1e-5):
    m = jnp.mean(x, axis=axis, keepdims=True)
    v = jnp.var(x, axis=axis, keepdims=True)
    return (x - m) / jnp.sqrt(v + eps)
def _scatter_add(tgt, idx, src, axis=0):
    return tgt.at[idx].add(src)
def _segment_sum(src, seg, n):
    return jax.ops.segment_sum(src, seg, n)
class _Rng:
    def __init__(self, key):
        self._k = key
    def _next(self):
        self._k, sub = jax.random.split(self._k)
        return sub
    def normal(self, shape):
        return jax.random.normal(self._next(), shape, dtype=jnp.bfloat16)
    def randint(self, lo, hi, shape):
        return jax.random.randint(self._next(), shape, lo, hi, dtype=jnp.int32)
    def uniform(self, shape, lo=0.0, hi=1.0):
        return jax.random.uniform(self._next(), shape, jnp.bfloat16, lo, hi)
    def permutation(self, n):
        return jax.random.permutation(self._next(), n)


kernel_name = 'gated_mix__compressed_kv_cla__ssm_conv_h3__prompt'

def setup_inputs():
    _rng = _Rng(jax.random.key(int.from_bytes(__import__("os").urandom(4), "little")))
    _w = (lambda a: (lambda t: t.astype(jnp.bfloat16) if jnp.issubdtype(t.dtype, jnp.floating) else t)(jnp.asarray(a)))
    def _A_setup():
        B, H, Sq, Sk, D, M = 1, 32, 2048, 2048, 128, 1024
        Dc = 4 * D
        return {
            "x": _w((lambda *s: _rng.normal(s) * 0.05)(B, Sq, M)),
            "c_kv": _w((lambda *s: _rng.normal(s) * 0.8)(B, Sk, Dc)),
            "w_q": _w((lambda *s: _rng.normal(s) * 3.2)(M, H, D) * (M ** -0.5)),
            "w_uk": _w((lambda *s: _rng.normal(s) * 3.2)(Dc, H, D) * (Dc ** -0.5)),
            "w_uv": _w((lambda *s: _rng.normal(s) * 0.8)(Dc, H, D) * (Dc ** -0.5)),
            "w_o": _w((lambda *s: _rng.normal(s) * 0.8)(H, D, M) * ((H * D) ** -0.5)),
        }
    _A_in = _A_setup()

    def _B_setup():
        B, S, D = 1, 2048, 1024
        ks = 4
        return {
            "q": _w((lambda *s: _rng.normal(s) * 0.05)(B, S, D)),
            "k": _w((lambda *s: _rng.normal(s) * 0.8)(B, S, D)),
            "v": _w((lambda *s: _rng.normal(s) * 0.8)(B, S, D)),
            "shift_k": _w((lambda *s: _rng.normal(s) * 0.8)(D, ks) * 0.5),
            "ssm_k": _w((lambda *s: _rng.normal(s) * 0.8)(D, S) * (1.0 / S ** 0.5)),
            "ssm_D": _w((lambda *s: _rng.normal(s) * 0.8)(D)),
        }
    _B_in = _B_setup()

    return {
        "A_x": _A_in["x"],
        "A_c_kv": _A_in["c_kv"],
        "A_w_q": _A_in["w_q"],
        "A_w_uk": _A_in["w_uk"],
        "A_w_uv": _A_in["w_uv"],
        "A_w_o": _A_in["w_o"],
        "B_q": _B_in["q"],
        "B_k": _B_in["k"],
        "B_v": _B_in["v"],
        "B_shift_k": _B_in["shift_k"],
        "B_ssm_k": _B_in["ssm_k"],
        "B_ssm_D": _B_in["ssm_D"],
        "gate_w": _w((lambda *s: _rng.normal(s) * 0.05)(1024) * 16.0),
    }

def reference(A_x, A_c_kv, A_w_q, A_w_uk, A_w_uv, A_w_o, B_q, B_k, B_v, B_shift_k, B_ssm_k, B_ssm_D, gate_w):
    def _A_ref(x, c_kv, w_q, w_uk, w_uv, w_o):
        B, Sq, M = x.shape[0], x.shape[1], x.shape[2]
        Sk = c_kv.shape[1]
        H, D = w_q.shape[1], w_q.shape[2]
        q = jnp.einsum("bqm,mhd->bhqd", x, w_q)
        k = jnp.einsum("bkc,chd->bhkd", c_kv, w_uk)
        v = jnp.einsum("bkc,chd->bhkd", c_kv, w_uv)
        scores = jnp.einsum("bhqd,bhkd->bhqk", q, k) * (D ** -0.5)
        off = Sk - Sq
        qi = jnp.arange(Sq)[:, None]
        kj = jnp.arange(Sk)[None, :]
        cmask = kj <= (qi + off)
        scores = jnp.where(cmask[None, None], scores, -1e9)
        p = _softmax(scores, axis=-1)
        ctx = jnp.einsum("bhqk,bhkd->bhqd", p, v)
        return jnp.einsum("bhqd,hdm->bqm", ctx, w_o)

    def _B_ref(q, k, v, shift_k, ssm_k, ssm_D):
        B, S, D = q.shape
        ks = shift_k.shape[-1]
        k_pad = jnp.pad(k, ((0, 0), (ks - 1, 0), (0, 0)))
        k_shift = jnp.zeros_like(k)
        for t in range(ks):
            k_shift = k_shift + k_pad[:, t:t + S, :] * shift_k[:, ks - 1 - t][None, None, :]
        kv = k_shift * v
        L = 2 * S
        kv_pad = jnp.pad(kv, ((0, 0), (0, S), (0, 0)))
        kf_pad = jnp.pad(ssm_k, ((0, 0), (0, S)))
        kv_f = (lambda x, axes=(-2,-1): jnp.fft.rfft2(x.astype(jnp.float32), axes=axes))(kv_pad[:, None, :, :], axes=(1, 2))
        kf_f = (lambda x, axes=(-2,-1): jnp.fft.rfft2(x.astype(jnp.float32), axes=axes))(kf_pad[:, None, :], axes=(1, 2))
        kf_f = (lambda x, *d: x.transpose(*d))(kf_f, 1, 2, 0)
        y_f = kv_f * kf_f[None, :, :, :]
        y = (lambda x, s, axes=(-2,-1): jnp.fft.irfft2(x, s=s, axes=axes).astype(jnp.bfloat16))(y_f, (1, L), axes=(1, 2))[:, 0, :S, :]
        y = y + kv * ssm_D[None, None, :]
        return q * y

    x = A_x
    g = _sigmoid((x * gate_w).sum(-1, keepdims=True))
    a = _A_ref(x, A_c_kv, A_w_q, A_w_uk, A_w_uv, A_w_o)
    b = _B_ref(x, B_k, B_v, B_shift_k, B_ssm_k, B_ssm_D)
    return g * a + (1 - g) * b
```

```python
import functools
import math

import jax
import jax.numpy as jnp
import numpy as np
from jax import lax
from jax.experimental import pallas as pl
from jax.experimental.pallas import tpu as pltpu

S, M, H, D, DC, KS = 2048, 1024, 32, 128, 512, 4
NP = H // 2
NG = M // 128
SB = 256
NE = 3
IL = 16
NS = 64
CH = 128
NCH = S // CH
KB = 3 * CH + 16
SH = S // 2
F32, BF16, U32 = jnp.float32, jnp.bfloat16, jnp.uint32

_ORDER = (
    "Q2 K3 s4a Q3 s4b p4a s5a K4 p4b s5b p5a s6a Q4 p5b s6b p6a s7a K5 p6b s7b p7a "
    "s8a Q5 p7b s8b p8a s9a K6 p8b s9b p9a s10a Q6 p9b s10b p10a s11a K7 p10b s11b p11a "
    "s12a Q7 p11b s12b p12a s13a p12b s13b p13a s14a p13b s14b p14a s15a p14b s15b p15a "
    "Q0 p15b s1 s0 Q1 p1 p0 s3 s2 p3 p2")


def _steps():
    steps = []
    for tok in _ORDER.split():
        if tok[0] in "KQ":
            steps.append((tok[0], int(tok[1:])))
        else:
            heads = {"a": (0,), "b": (1,)}.get(tok[-1])
            blk = int(tok[1:-1] if heads else tok[1:])
            steps += [(tok[0], h, blk) for h in heads or (0, 1)]
    return steps


def _dft_matrices():
    even = np.arange(0, CH, 2)
    f = np.concatenate([even, CH - 1 - even]).astype(np.float64)
    ang = (np.pi * (f + 0.5) / CH)[:, None] * np.arange(CH)[None, :]
    fwd = np.concatenate([np.cos(ang), -np.sin(ang)], axis=0)
    inv = np.concatenate([np.cos(ang[:CH // 2]).T, -np.sin(ang[:CH // 2]).T], axis=1) / CH
    inv = np.concatenate([inv[0::2], inv[1::2]], axis=0)
    return fwd.astype(np.dtype(BF16)), inv.astype(np.dtype(BF16))


_FWD, _INV = _dft_matrices()


def _dot(a, b):
    return jnp.dot(a, b, preferred_element_type=F32)


def _dot_nt(a, b):
    return lax.dot_general(a, b, (((1,), (1,)), ((), ())), preferred_element_type=F32)


def _rows(ref, r, n):
    return pltpu.bitcast(ref[r // 2:(r + n) // 2, :], BF16).astype(F32)


def _halves(w):
    return pltpu.bitcast(w << 16, F32), pltpu.bitcast(w & np.uint32(0xFFFF0000), F32)


def _lhs_term(p, a):
    return (lambda: a(0, 0) + a(1, 1), lambda: a(1, 0) + a(1, 1), lambda: a(0, 0),
            lambda: a(1, 1), lambda: a(0, 0) + a(0, 1), lambda: a(1, 0) - a(0, 0),
            lambda: a(0, 1) - a(1, 1))[p]()


def _rhs_term(p, b):
    return (lambda: b(0, 0) + b(1, 1), lambda: b(0, 0), lambda: b(0, 1) - b(1, 1),
            lambda: b(1, 0) - b(0, 0), lambda: b(1, 1), lambda: b(0, 0) + b(0, 1),
            lambda: b(1, 0) + b(1, 1))[p]()


def _strassen(prod):
    m2, m4 = prod(1), prod(3)
    c21 = m2 + m4
    m1 = prod(0)
    c22 = m1 - m2 + prod(5)
    c11 = m1 + m4 + prod(6)
    m3 = prod(2)
    c22 = c22 + m3
    m5 = prod(4)

    def merge(top, bot):
        return jnp.concatenate(
            [v[r:r + IL] for r in range(0, top.shape[0], IL) for v in (top, bot)], axis=0)
    return merge(c11 - m5, c21), merge(m3 + m5, c22)


def _zeros_like_index(i, n):
    return [lax.shift_right_logical(i, 5 + k) for k in range(n)]


def _kernel(x_hbm, c_hbm, wq_hbm, wk_hbm, wv_hbm, wo_hbm, bk_hbm, bv_hbm, sk_hbm,
            shift_hbm, dd_hbm, gw_hbm, fwd_hbm, inv_hbm, out_hbm,
            x_s, c_s, wkv_s, wq_s, wo_s, bk_s, bv_s, xg_s, sk_s,
            ctx_s, kve_s, kv_s, s_s, g_s, skip_s, a_s, b_s, f_s, y_s,
            even_s, top_s, bot_s, par_s, fwd_s, inv_s, shift_s, dd_s, gw_s,
            wkv_sems, in_sems, late_sems, out_sems):
    head, rest = pl.ds(0, NE * SB), pl.ds(NE * SB, S - NE * SB)
    copies = [pltpu.make_async_copy(h, v, in_sems.at[n]) for n, (h, v) in enumerate((
        (gw_hbm, gw_s), (shift_hbm, shift_s), (dd_hbm, dd_s), (fwd_hbm, fwd_s),
        (inv_hbm, inv_s), (c_hbm.at[head], c_s.at[0, head]),
        (c_hbm.at[rest], c_s.at[0, rest]), (x_hbm, x_s.at[0])))]
    first, second = copies[:6], copies[6:]
    wq_sem = in_sems.at[len(copies)]

    def start_wkv(pairs):
        for j in pairs:
            for h, off in ((wk_hbm, 0), (wv_hbm, DC)):
                pltpu.make_async_copy(h.bitcast(U32).at[:, j, :], wkv_s.at[j, pl.ds(off, DC)],
                                      wkv_sems.at[j // 2]).start()

    for cp in first:
        cp.start()
    start_wkv(range(2))
    a_s[...] = jnp.zeros((SH, 128), F32)
    b_s[1] = jnp.zeros((S, 128), F32)
    par_s[...] = jnp.zeros(par_s.shape, F32)
    for cp in first:
        cp.wait()
    start_wkv(range(2, NP))
    shift, dd = shift_s[...].astype(F32), dd_s[...].astype(F32)
    for g in range(NG):
        par_s[g, 0:KS, :] = shift[:, g * 128:(g + 1) * 128]
        par_s[g, KS:KS + 1, :] = dd[g:g + 1, :]

    def weight_terms(w):
        n = w.shape[0] // 2
        heads = _halves(w)
        return [_rhs_term(p, lambda k, h: heads[h][k * n:(k + 1) * n]) for p in range(7)]

    def kv_weights(j):
        return [jnp.concatenate(kv, axis=1).astype(BF16) for kv in zip(
            weight_terms(wkv_s[j, 0:DC]), weight_terms(wkv_s[j, DC:2 * DC]))]

    def project(in_s, zs, r, n, w):
        hw = in_s.shape[2] // 2

        def prod(p):
            def block(i, k):
                return jnp.concatenate(
                    [in_s[zs[p], q + i * IL:q + (i + 1) * IL, k * hw:(k + 1) * hw].astype(F32)
                     for q in range(r, r + n, 2 * IL)], axis=0)
            return _dot(_lhs_term(p, block).astype(BF16), w[p])
        return _strassen(prod)

    def project_kv(zs, r, n, w, dst, r0):
        for h, kv in enumerate(project(c_s, zs, r, n, w)):
            dst[h, r0:r0 + n, :] = kv[:, 0:D].astype(BF16)
            dst[2 + h, r0:r0 + n, :] = kv[:, D:2 * D].astype(BF16)

    def warm_up(t, carry):
        @pl.when(t == 1)
        def _():
            for cp in second:
                cp.start()
            for j in range(NP):
                pltpu.make_async_copy(wq_hbm.bitcast(U32).at[:, j, :], wq_s.at[j], wq_sem).start()

        two = wkv_s.at[pl.ds(2 * t, 2)]
        pltpu.make_async_copy(two, two, wkv_sems.at[t]).wait()
        s_s[t, 0:8, :] = jnp.zeros((8, 128), F32)
        zs = _zeros_like_index(t, 14)
        for n in range(2):
            j = 2 * t + n
            project_kv(zs[7 * n:], 0, NE * SB, kv_weights(j), kve_s.at[j], 0)
        return carry

    lax.fori_loop(0, NP // 2, warm_up, 0)
    for cp in second:
        cp.wait()
    pltpu.make_async_copy(wq_s, wq_s, wq_sem).wait()

    late = ((wo_hbm, wo_s), (bk_hbm, bk_s), (bv_hbm, bv_s), (x_hbm, xg_s))
    for g in range(NG):
        lanes = pl.ds(g * 128, 128)
        for n, (h, v) in enumerate(late):
            pltpu.make_async_copy(h.bitcast(U32).at[:, lanes], v.at[g], late_sems.at[n]).start()
        pltpu.make_async_copy(sk_hbm.at[lanes], sk_s.at[g], late_sems.at[len(late)]).start()

    q_scale = D ** -0.5 * math.log2(math.e)
    causal = (lax.broadcasted_iota(jnp.int32, (128, 128), 1)
              <= lax.broadcasted_iota(jnp.int32, (128, 128), 0))

    def pair(j, carry):
        zs = _zeros_like_index(j, 7)
        gw = gw_s[...].astype(F32)
        rows = pl.ds(pl.multiple_of(j * (S // NP), S // NP), S // NP)
        logit = jnp.sum(functools.reduce(jnp.add, [
            x_s[0, rows, g * 128:(g + 1) * 128].astype(F32) * gw[g:g + 1, :]
            for g in range(NG)]), axis=1, keepdims=True)
        g_s[rows, :] = jnp.broadcast_to(jax.nn.sigmoid(logit), (S // NP, 128))

        wkv = kv_weights(j)
        wq = [v.astype(BF16) for v in weight_terms(wq_s[j])]

        def cache(idx, n):
            if n <= NE * SB:
                return kve_s[j, idx, 0:n, :]
            return jnp.concatenate([kve_s[j, idx], kv_s[idx, 0:n - NE * SB, :]], axis=0)

        qs, scores, ctx = {}, {}, {}
        slot = 0
        for step in _steps():
            if step[0] == "K":
                project_kv(zs, step[1] * SB, SB, wkv, kv_s, (step[1] - NE) * SB)
            elif step[0] == "Q":
                for h, q in enumerate(project(x_s, zs, step[1] * SB, SB, wq)):
                    for u in range(2):
                        qs[h, 2 * step[1] + u] = (q[u * 128:(u + 1) * 128] * q_scale).astype(BF16)
            elif step[0] == "s":
                _, h, i = step
                s = _dot_nt(qs.pop((h, i)), cache(h, (i + 1) * 128))
                tiles = [s[:, c * 128:(c + 1) * 128] for c in range(i + 1)]
                tiles[i] = jnp.where(causal, tiles[i], -1e30)
                row_max = jnp.max(functools.reduce(jnp.maximum, tiles), axis=1, keepdims=True)
                for c in range(i + 1):
                    s_s[(slot + c) % NS, 0:128, :] = tiles[c]
                scores[h, i] = (row_max, slot)
                slot += i + 1
            else:
                _, h, i = step
                row_max, start = scores.pop((h, i))
                assert slot - start <= NS
                ps = [jnp.exp2(s_s[(start + c) % NS, 0:128, :] - row_max) for c in range(i + 1)]
                total = functools.reduce(jnp.add, ps)
                if i:
                    ps[i] = jnp.minimum(ps[i], total)
                inv_l = pltpu.reciprocal(jnp.sum(total, axis=1, keepdims=True), full_range=False)
                ctx[h, i] = inv_l * _dot(jnp.concatenate(ps, axis=1).astype(BF16),
                                         cache(2 + h, (i + 1) * 128))
                if (1 - h, i) in ctx:
                    both = (ctx.pop((0, i)), ctx.pop((1, i)))
                    blocks = [[jnp.concatenate(
                        [o[r + n * IL:r + (n + 1) * IL] for r in range(0, 128, 2 * IL)], axis=0)
                        for o in both] for n in range(2)]
                    r = (i % 8) * 64
                    for p in range(7):
                        ctx_s[p, i // 8, j, r:r + 64, :] = _lhs_term(
                            p, lambda n, k: blocks[n][k]).astype(BF16)
        return carry

    lax.fori_loop(0, NP, pair, 0)
    for n, v in enumerate([v for _, v in late] + [sk_s]):
        pltpu.make_async_copy(v, v, late_sems.at[n]).wait()

    def out_copy(part, g):
        half = g % 2
        col, row = (g - half, half * SH) if part == 0 else (g, (part - 1) * SH)
        src = (even_s, top_s, bot_s)[part].at[g if part == 0 else g // 2]
        dst = out_hbm.at[pl.ds(pl.multiple_of(row, SH), SH),
                         pl.ds(pl.multiple_of(col * 128, 128), 128)]
        return pltpu.make_async_copy(src, dst, out_sems.at[part])

    def group(g, carry):
        zs = _zeros_like_index(g, NCH + 2)
        z_st, z_ld = zs[NCH], zs[NCH + 1]
        half = lax.bitwise_and(g, 1)
        g0 = g - half
        par = par_s[g]
        hc = CH // 2

        def spectra():
            fwd = fwd_s[...]
            k_tail, prev = jnp.zeros((8, 128), F32), None
            for c in range(NCH):
                r = c * CH
                k = _rows(bk_s.at[g], r, CH)
                ext = jnp.concatenate([k_tail, k], axis=0)
                k_tail = k[CH - 8:CH]
                shifted = k * par[0:1, :]
                for t in range(1, KS):
                    shifted = shifted + pltpu.roll(ext, t, 0)[8:8 + CH] * par[t:t + 1, :]
                kv = shifted * _rows(bv_s.at[g], r, CH)
                skip_s[z_st, r:r + CH, :] = kv * par[KS:KS + 1, :]
                u = _dot(fwd, kv.astype(BF16))
                f_s[z_st, c, 0:2 * CH, :] = u
                f_s[z_st, c, 2 * CH:3 * CH, :] = u[0:CH] + u[CH:2 * CH]
                cur = _dot_nt(fwd, sk_s[g, :, r:r + CH])
                if prev is None:
                    re, im = cur[0:CH], cur[CH:2 * CH]
                else:
                    re = jnp.concatenate([cur[0:hc] - prev[CH:CH + hc],
                                          cur[hc:CH] + prev[CH + hc:2 * CH]], axis=0)
                    im = jnp.concatenate([cur[CH:CH + hc] + prev[0:hc],
                                          cur[CH + hc:2 * CH] - prev[hc:CH]], axis=0)
                f_s[z_st, c, KB:KB + CH, :] = im - re
                f_s[z_st, c, KB + CH:KB + 2 * CH, :] = im + re
                f_s[z_st, c, KB + 2 * CH:KB + 3 * CH, :] = re
                prev = cur
                yield

        def convolve():
            for i in range(NCH):
                acc = [functools.reduce(jnp.add, [
                    f_s[zs[i], c, o:o + CH, :] * f_s[zs[i], i - c, KB + o:KB + o + CH, :]
                    for c in range(i + 1)]) for o in (0, CH, 2 * CH)]
                re, im = acc[2] - acc[1], acc[2] + acc[0]
                y_s[i] = jnp.concatenate(
                    [re[:hc] + re[hc:], im[:hc] - im[hc:],
                     re[:hc] - re[hc:], im[:hc] + im[hc:]], axis=0).astype(BF16)
            for c in range(NCH):
                for odd, x in enumerate(_halves(xg_s[g, c * hc:(c + 1) * hc, :])):
                    steps = pl.ds(c * CH + odd, hc, stride=2)
                    y = _dot(inv_s[odd * hc:(odd + 1) * hc, :], y_s[c, odd * CH:(odd + 1) * CH, :])
                    y = y + skip_s[z_ld, steps, :]
                    b_s[half, steps, :] = (1.0 - g_s[steps, :]) * (x * y)
                yield

        forward, backward = spectra(), convolve()
        extra = [[] for _ in range(7 * NP // 4)]
        for c in range(NCH):
            extra[2 + c // 4].append(forward)
            extra[20 + c // 4].append(backward)

        def prod(p):
            acc = []
            for j0 in range(0, NP, 4):
                for chunk in extra.pop(0):
                    next(chunk)
                js = range(j0, j0 + 4)
                lhs = jnp.concatenate([ctx_s[p, half, j] for j in js], axis=1)
                rhs = _rhs_term(p, lambda k, n: jnp.concatenate(
                    [_rows(wo_s.at[g0 + n + zs[p]], (2 * j + k) * D, D) for j in js], axis=0))
                acc.append(_dot(lhs, rhs.astype(BF16)))
            return functools.reduce(jnp.add, acc)

        rows = pl.ds(pl.multiple_of(half * SH, SH), SH)
        a0, a1 = [g_s[rows, :] * a for a in _strassen(prod)]
        gp = lax.shift_right_logical(g, 1)
        top_s[gp] = (a_s[...] + b_s[1, 0:SH, :]).astype(BF16)
        bot_s[gp] = (a1 + b_s[1, SH:S, :]).astype(BF16)
        even_s[g] = (a0 + b_s[0, rows, :]).astype(BF16)
        a_s[...] = a1
        out_copy(0, g).start()

        @pl.when(half == 1)
        def _():
            out_copy(1, g).start()
            out_copy(2, g).start()
        return carry

    lax.fori_loop(0, NG, group, 0)
    for g in range(NG):
        for part in range(3 if g % 2 else 1):
            out_copy(part, g).wait()


@jax.jit
def pallas_gated_mix__compressed_kv_cla__ssm_conv_h3__prompt_kernel(
    A_x: jax.Array,
    A_c_kv: jax.Array,
    A_w_q: jax.Array,
    A_w_uk: jax.Array,
    A_w_uv: jax.Array,
    A_w_o: jax.Array,
    B_q: jax.Array,
    B_k: jax.Array,
    B_v: jax.Array,
    B_shift_k: jax.Array,
    B_ssm_k: jax.Array,
    B_ssm_D: jax.Array,
    gate_w: jax.Array,
):
    del B_q
    hbm = pl.BlockSpec(memory_space=pl.ANY)
    out = pl.pallas_call(
        _kernel,
        out_shape=jax.ShapeDtypeStruct((S, M), BF16),
        in_specs=[hbm] * 14,
        out_specs=hbm,
        scratch_shapes=[
            pltpu.VMEM((1, S, M), BF16),
            pltpu.VMEM((1, S, DC), BF16),
            pltpu.VMEM((NP, 2 * DC, D), U32),
            pltpu.VMEM((NP, M, D), U32),
            pltpu.VMEM((NG, H * D // 2, 128), U32),
            pltpu.VMEM((NG, S // 2, 128), U32),
            pltpu.VMEM((NG, S // 2, 128), U32),
            pltpu.VMEM((NG, S // 2, 128), U32),
            pltpu.VMEM((NG, 128, S), BF16),
            pltpu.VMEM((7, 2, NP, S // 4, D), BF16),
            pltpu.VMEM((NP, 4, NE * SB, D), BF16),
            pltpu.VMEM((4, S - NE * SB, D), BF16),
            pltpu.VMEM((NS, 136, 128), F32),
            pltpu.VMEM((S, 128), F32),
            pltpu.VMEM((1, S, 128), F32),
            pltpu.VMEM((SH, 128), F32),
            pltpu.VMEM((2, S, 128), F32),
            pltpu.VMEM((1, NCH, 6 * CH + 32, 128), F32),
            pltpu.VMEM((NCH, 2 * CH, 128), BF16),
            pltpu.VMEM((NG, SH, 128), BF16),
            pltpu.VMEM((NG // 2, SH, 128), BF16),
            pltpu.VMEM((NG // 2, SH, 128), BF16),
            pltpu.VMEM((NG, 8, 128), F32),
            pltpu.VMEM((2 * CH, CH), BF16),
            pltpu.VMEM((CH, CH), BF16),
            pltpu.VMEM((KS, M), BF16),
            pltpu.VMEM((NG, 128), BF16),
            pltpu.VMEM((NG, 128), BF16),
            pltpu.SemaphoreType.DMA((NP // 2,)),
            pltpu.SemaphoreType.DMA((9,)),
            pltpu.SemaphoreType.DMA((5,)),
            pltpu.SemaphoreType.DMA((3,)),
        ],
        compiler_params=pltpu.CompilerParams(vmem_limit_bytes=122 * 2**20),
    )(A_x.reshape(S, M), A_c_kv.reshape(S, DC), A_w_q, A_w_uk, A_w_uv,
      A_w_o.reshape(H * D, M), B_k.reshape(S, M), B_v.reshape(S, M), B_ssm_k,
      B_shift_k.T, B_ssm_D.reshape(NG, 128), gate_w.reshape(NG, 128), _FWD, _INV)
    return out.reshape(1, S, M)
```

```python
import functools
import math

import jax
import jax.numpy as jnp
import numpy as np
from jax import lax
from jax.experimental import pallas as pl
from jax.experimental.pallas import tpu as pltpu

S, M, H, D, DC, KS = 2048, 1024, 32, 128, 512, 4
NP = H // 2
NG = M // 128
SB = 256
NE = 3
IL = 16
NS = 64
CH = 128
NCH = S // CH
KB = 3 * CH + 16
SH = S // 2
F32, BF16, U32 = jnp.float32, jnp.bfloat16, jnp.uint32

_ORDER = (
    "Q2 K3 s4a Q3 s4b p4a s5a K4 p4b s5b p5a s6a Q4 p5b s6b p6a s7a K5 p6b s7b p7a "
    "s8a Q5 p7b s8b p8a s9a K6 p8b s9b p9a s10a Q6 p9b s10b p10a s11a K7 p10b s11b p11a "
    "s12a Q7 p11b s12b p12a s13a p12b s13b p13a s14a p13b s14b p14a s15a p14b s15b p15a "
    "Q0 p15b s1 s0 Q1 p1 p0 s3 s2 p3 p2")


def _steps():
    steps = []
    for tok in _ORDER.split():
        if tok[0] in "KQ":
            steps.append((tok[0], int(tok[1:])))
        else:
            heads = {"a": (0,), "b": (1,)}.get(tok[-1])
            blk = int(tok[1:-1] if heads else tok[1:])
            steps += [(tok[0], h, blk) for h in heads or (0, 1)]
    return steps


def _dft_matrices():
    even = np.arange(0, CH, 2)
    f = np.concatenate([even, CH - 1 - even]).astype(np.float64)
    ang = (np.pi * (f + 0.5) / CH)[:, None] * np.arange(CH)[None, :]
    fwd = np.concatenate([np.cos(ang), -np.sin(ang)], axis=0)
    inv = np.concatenate([np.cos(ang[:CH // 2]).T, -np.sin(ang[:CH // 2]).T], axis=1) / CH
    inv = np.concatenate([inv[0::2], inv[1::2]], axis=0)
    return fwd.astype(np.dtype(BF16)), inv.astype(np.dtype(BF16))


_FWD, _INV = _dft_matrices()


def _dot(a, b):
    return jnp.dot(a, b, preferred_element_type=F32)


def _dot_nt(a, b):
    return lax.dot_general(a, b, (((1,), (1,)), ((), ())), preferred_element_type=F32)


def _rows(ref, r, n):
    return pltpu.bitcast(ref[r // 2:(r + n) // 2, :], BF16).astype(F32)


def _halves(w):
    return pltpu.bitcast(w << 16, F32), pltpu.bitcast(w & np.uint32(0xFFFF0000), F32)


def _lhs_term(p, a):
    return (lambda: a(0, 0) + a(1, 1), lambda: a(1, 0) + a(1, 1), lambda: a(0, 0),
            lambda: a(1, 1), lambda: a(0, 0) + a(0, 1), lambda: a(1, 0) - a(0, 0),
            lambda: a(0, 1) - a(1, 1))[p]()


def _rhs_term(p, b):
    return (lambda: b(0, 0) + b(1, 1), lambda: b(0, 0), lambda: b(0, 1) - b(1, 1),
            lambda: b(1, 0) - b(0, 0), lambda: b(1, 1), lambda: b(0, 0) + b(0, 1),
            lambda: b(1, 0) + b(1, 1))[p]()


def _strassen(prod):
    m2, m4 = prod(1), prod(3)
    c21 = m2 + m4
    m1 = prod(0)
    c22 = m1 - m2 + prod(5)
    c11 = m1 + m4 + prod(6)
    m3 = prod(2)
    c22 = c22 + m3
    m5 = prod(4)

    def merge(top, bot):
        return jnp.concatenate(
            [v[r:r + IL] for r in range(0, top.shape[0], IL) for v in (top, bot)], axis=0)
    return merge(c11 - m5, c21), merge(m3 + m5, c22)


def _zeros_like_index(i, n):
    return [lax.shift_right_logical(i, 5 + k) for k in range(n)]


def _kernel(x_hbm, c_hbm, wq_hbm, wk_hbm, wv_hbm, wo_hbm, bk_hbm, bv_hbm, sk_hbm,
            shift_hbm, dd_hbm, gw_hbm, fwd_hbm, inv_hbm, out_hbm,
            x_s, c_s, wkv_s, wq_s, wo_s, bk_s, bv_s, xg_s, sk_s,
            ctx_s, kve_s, kv_s, s_s, g_s, skip_s, a_s, b_s, f_s, y_s,
            even_s, top_s, bot_s, par_s, fwd_s, inv_s, shift_s, dd_s, gw_s,
            in_sems, late_sems, out_sems):
    head, rest = pl.ds(0, NE * SB), pl.ds(NE * SB, S - NE * SB)
    copies = [pltpu.make_async_copy(h, v, in_sems.at[n]) for n, (h, v) in enumerate((
        (gw_hbm, gw_s), (shift_hbm, shift_s), (dd_hbm, dd_s), (fwd_hbm, fwd_s),
        (inv_hbm, inv_s), (c_hbm.at[head], c_s.at[0, head]),
        (c_hbm.at[rest], c_s.at[0, rest]), (x_hbm, x_s.at[0])))]
    first, second = copies[:6], copies[6:]
    wq_sem = in_sems.at[len(copies)]
    wkv_sem = len(copies) + 1

    for cp in first:
        cp.start()
    for j in range(NP):
        for h, off in ((wk_hbm, 0), (wv_hbm, DC)):
            pltpu.make_async_copy(h.bitcast(U32).at[:, j, :], wkv_s.at[j, pl.ds(off, DC)],
                                  in_sems.at[wkv_sem + j // 2]).start()
    for cp in second:
        cp.start()
    for j in range(NP):
        pltpu.make_async_copy(wq_hbm.bitcast(U32).at[:, j, :], wq_s.at[j], wq_sem).start()

    a_s[...] = jnp.zeros((SH, 128), F32)
    b_s[...] = jnp.zeros(b_s.shape, F32)
    par_s[...] = jnp.zeros(par_s.shape, F32)
    for cp in first:
        cp.wait()
    shift, dd = shift_s[...].astype(F32), dd_s[...].astype(F32)
    for g in range(NG):
        par_s[g, 0:KS, :] = shift[:, g * 128:(g + 1) * 128]
        par_s[g, KS:KS + 1, :] = dd[g:g + 1, :]

    def weight_terms(w):
        n = w.shape[0] // 2
        heads = _halves(w)
        return [_rhs_term(p, lambda k, h: heads[h][k * n:(k + 1) * n]) for p in range(7)]

    def kv_weights(j):
        return [jnp.concatenate(kv, axis=1).astype(BF16) for kv in zip(
            weight_terms(wkv_s[j, 0:DC]), weight_terms(wkv_s[j, DC:2 * DC]))]

    def project(in_s, zs, r, n, w):
        hw = in_s.shape[2] // 2

        def prod(p):
            def block(i, k):
                return jnp.concatenate(
                    [in_s[zs[p], q + i * IL:q + (i + 1) * IL, k * hw:(k + 1) * hw].astype(F32)
                     for q in range(r, r + n, 2 * IL)], axis=0)
            return _dot(_lhs_term(p, block).astype(BF16), w[p])
        return _strassen(prod)

    def project_kv(zs, r, n, w, dst, r0):
        for h, kv in enumerate(project(c_s, zs, r, n, w)):
            dst[h, r0:r0 + n, :] = kv[:, 0:D].astype(BF16)
            dst[2 + h, r0:r0 + n, :] = kv[:, D:2 * D].astype(BF16)

    def warm_up(t, carry):
        two = wkv_s.at[pl.ds(2 * t, 2)]
        pltpu.make_async_copy(two, two, in_sems.at[wkv_sem + t]).wait()
        s_s[t, 0:8, :] = jnp.zeros((8, 128), F32)
        zs = _zeros_like_index(t, 14)
        for n in range(2):
            j = 2 * t + n
            project_kv(zs[7 * n:], 0, NE * SB, kv_weights(j), kve_s.at[j], 0)
        return carry

    lax.fori_loop(0, NP // 2, warm_up, 0)
    for cp in second:
        cp.wait()
    pltpu.make_async_copy(wq_s, wq_s, wq_sem).wait()

    late = ((wo_hbm, wo_s), (bk_hbm, bk_s), (bv_hbm, bv_s), (x_hbm, xg_s))
    for g in range(NG):
        lanes = pl.ds(g * 128, 128)
        for n, (h, v) in enumerate(late):
            pltpu.make_async_copy(h.bitcast(U32).at[:, lanes], v.at[g], late_sems.at[n]).start()
        pltpu.make_async_copy(sk_hbm.at[lanes], sk_s.at[g], late_sems.at[len(late)]).start()

    q_scale = D ** -0.5 * math.log2(math.e)
    causal = (lax.broadcasted_iota(jnp.int32, (128, 128), 1)
              <= lax.broadcasted_iota(jnp.int32, (128, 128), 0))

    def pair(j, carry):
        zs = _zeros_like_index(j, 7)
        gw = gw_s[...].astype(F32)
        rows = pl.ds(pl.multiple_of(j * (S // NP), S // NP), S // NP)
        logit = jnp.sum(functools.reduce(jnp.add, [
            x_s[0, rows, g * 128:(g + 1) * 128].astype(F32) * gw[g:g + 1, :]
            for g in range(NG)]), axis=1, keepdims=True)
        g_s[rows, :] = jnp.broadcast_to(jax.nn.sigmoid(logit), (S // NP, 128))

        wkv = kv_weights(j)
        wq = [v.astype(BF16) for v in weight_terms(wq_s[j])]

        def cache(idx, n):
            if n <= NE * SB:
                return kve_s[j, idx, 0:n, :]
            return jnp.concatenate([kve_s[j, idx], kv_s[idx, 0:n - NE * SB, :]], axis=0)

        qs, scores, ctx = {}, {}, {}
        slot = 0
        for step in _steps():
            if step[0] == "K":
                project_kv(zs, step[1] * SB, SB, wkv, kv_s, (step[1] - NE) * SB)
            elif step[0] == "Q":
                for h, q in enumerate(project(x_s, zs, step[1] * SB, SB, wq)):
                    for u in range(2):
                        qs[h, 2 * step[1] + u] = (q[u * 128:(u + 1) * 128] * q_scale).astype(BF16)
            elif step[0] == "s":
                _, h, i = step
                s = _dot_nt(qs.pop((h, i)), cache(h, (i + 1) * 128))
                tiles = [s[:, c * 128:(c + 1) * 128] for c in range(i + 1)]
                tiles[i] = jnp.where(causal, tiles[i], -1e30)
                row_max = jnp.max(functools.reduce(jnp.maximum, tiles), axis=1, keepdims=True)
                for c in range(i + 1):
                    s_s[(slot + c) % NS, 0:128, :] = tiles[c]
                scores[h, i] = (row_max, slot)
                slot += i + 1
            else:
                _, h, i = step
                row_max, start = scores.pop((h, i))
                assert slot - start <= NS
                ps = [jnp.exp2(s_s[(start + c) % NS, 0:128, :] - row_max) for c in range(i + 1)]
                total = functools.reduce(jnp.add, ps)
                if i:
                    ps[i] = jnp.minimum(ps[i], total)
                inv_l = pltpu.reciprocal(jnp.sum(total, axis=1, keepdims=True), full_range=False)
                ctx[h, i] = inv_l * _dot(jnp.concatenate(ps, axis=1).astype(BF16),
                                         cache(2 + h, (i + 1) * 128))
                if (1 - h, i) in ctx:
                    both = (ctx.pop((0, i)), ctx.pop((1, i)))
                    blocks = [[jnp.concatenate(
                        [o[r + n * IL:r + (n + 1) * IL] for r in range(0, 128, 2 * IL)], axis=0)
                        for o in both] for n in range(2)]
                    r = (i % 8) * 64
                    for p in range(7):
                        ctx_s[p, i // 8, j, r:r + 64, :] = _lhs_term(
                            p, lambda n, k: blocks[n][k]).astype(BF16)
        return carry

    lax.fori_loop(0, NP, pair, 0)
    for n, v in enumerate([v for _, v in late] + [sk_s]):
        pltpu.make_async_copy(v, v, late_sems.at[n]).wait()

    def out_copy(part, g):
        half = g % 2
        col, row = (g - half, half * SH) if part == 0 else (g, (part - 1) * SH)
        src = (even_s, top_s, bot_s)[part].at[g if part == 0 else g // 2]
        dst = out_hbm.at[pl.ds(pl.multiple_of(row, SH), SH),
                         pl.ds(pl.multiple_of(col * 128, 128), 128)]
        return pltpu.make_async_copy(src, dst, out_sems.at[part])

    def group(g, carry):
        zs = _zeros_like_index(g, NCH + 2)
        z_st, z_ld = zs[NCH], zs[NCH + 1]
        half = lax.bitwise_and(g, 1)
        g0 = g - half
        par = par_s[g]
        hc = CH // 2

        def spectra():
            fwd = fwd_s[...]
            k_tail, prev = jnp.zeros((8, 128), F32), None
            for c in range(NCH):
                r = c * CH
                k = _rows(bk_s.at[g], r, CH)
                ext = jnp.concatenate([k_tail, k], axis=0)
                k_tail = k[CH - 8:CH]
                shifted = k * par[0:1, :]
                for t in range(1, KS):
                    shifted = shifted + pltpu.roll(ext, t, 0)[8:8 + CH] * par[t:t + 1, :]
                kv = shifted * _rows(bv_s.at[g], r, CH)
                skip_s[z_st, r:r + CH, :] = kv * par[KS:KS + 1, :]
                u = _dot(fwd, kv.astype(BF16))
                f_s[z_st, c, 0:2 * CH, :] = u
                f_s[z_st, c, 2 * CH:3 * CH, :] = u[0:CH] + u[CH:2 * CH]
                cur = _dot_nt(fwd, sk_s[g, :, r:r + CH])
                if prev is None:
                    re, im = cur[0:CH], cur[CH:2 * CH]
                else:
                    re = jnp.concatenate([cur[0:hc] - prev[CH:CH + hc],
                                          cur[hc:CH] + prev[CH + hc:2 * CH]], axis=0)
                    im = jnp.concatenate([cur[CH:CH + hc] + prev[0:hc],
                                          cur[CH + hc:2 * CH] - prev[hc:CH]], axis=0)
                f_s[z_st, c, KB:KB + CH, :] = im - re
                f_s[z_st, c, KB + CH:KB + 2 * CH, :] = im + re
                f_s[z_st, c, KB + 2 * CH:KB + 3 * CH, :] = re
                prev = cur
                yield

        def convolve():
            for i in range(NCH):
                acc = [functools.reduce(jnp.add, [
                    f_s[zs[i], c, o:o + CH, :] * f_s[zs[i], i - c, KB + o:KB + o + CH, :]
                    for c in range(i + 1)]) for o in (0, CH, 2 * CH)]
                re, im = acc[2] - acc[1], acc[2] + acc[0]
                y_s[i] = jnp.concatenate(
                    [re[:hc] + re[hc:], im[:hc] - im[hc:],
                     re[:hc] - re[hc:], im[:hc] + im[hc:]], axis=0).astype(BF16)
            for c in range(NCH):
                for odd, x in enumerate(_halves(xg_s[g, c * hc:(c + 1) * hc, :])):
                    steps = pl.ds(c * CH + odd, hc, stride=2)
                    y = _dot(inv_s[odd * hc:(odd + 1) * hc, :], y_s[c, odd * CH:(odd + 1) * CH, :])
                    y = y + skip_s[z_ld, steps, :]
                    b_s[half, steps, :] = (1.0 - g_s[steps, :]) * (x * y)
                yield

        forward, backward = spectra(), convolve()
        extra = [[] for _ in range(7 * NP // 4)]
        for c in range(NCH):
            extra[2 + c // 4].append(forward)
            extra[20 + c // 4].append(backward)

        def prod(p):
            acc = []
            for j0 in range(0, NP, 4):
                for chunk in extra.pop(0):
                    next(chunk)
                js = range(j0, j0 + 4)
                lhs = jnp.concatenate([ctx_s[p, half, j] for j in js], axis=1)
                rhs = _rhs_term(p, lambda k, n: jnp.concatenate(
                    [_rows(wo_s.at[g0 + n + zs[p]], (2 * j + k) * D, D) for j in js], axis=0))
                acc.append(_dot(lhs, rhs.astype(BF16)))
            return functools.reduce(jnp.add, acc)

        rows = pl.ds(pl.multiple_of(half * SH, SH), SH)
        a0, a1 = [g_s[rows, :] * a for a in _strassen(prod)]
        gp = lax.shift_right_logical(g, 1)
        top_s[gp] = (a_s[...] + b_s[1, 0:SH, :]).astype(BF16)
        bot_s[gp] = (a1 + b_s[1, SH:S, :]).astype(BF16)
        even_s[g] = (a0 + b_s[0, rows, :]).astype(BF16)
        a_s[...] = a1
        out_copy(0, g).start()

        @pl.when(half == 1)
        def _():
            out_copy(1, g).start()
            out_copy(2, g).start()
        return carry

    lax.fori_loop(0, NG, group, 0)
    for g in range(NG):
        for part in range(3 if g % 2 else 1):
            out_copy(part, g).wait()


@jax.jit
def pallas_gated_mix__compressed_kv_cla__ssm_conv_h3__prompt_kernel(
    A_x: jax.Array,
    A_c_kv: jax.Array,
    A_w_q: jax.Array,
    A_w_uk: jax.Array,
    A_w_uv: jax.Array,
    A_w_o: jax.Array,
    B_q: jax.Array,
    B_k: jax.Array,
    B_v: jax.Array,
    B_shift_k: jax.Array,
    B_ssm_k: jax.Array,
    B_ssm_D: jax.Array,
    gate_w: jax.Array,
):
    del B_q
    hbm = pl.BlockSpec(memory_space=pl.ANY)
    out = pl.pallas_call(
        _kernel,
        out_shape=jax.ShapeDtypeStruct((S, M), BF16),
        in_specs=[hbm] * 14,
        out_specs=hbm,
        scratch_shapes=[
            pltpu.VMEM((1, S, M), BF16),
            pltpu.VMEM((1, S, DC), BF16),
            pltpu.VMEM((NP, 2 * DC, D), U32),
            pltpu.VMEM((NP, M, D), U32),
            pltpu.VMEM((NG, H * D // 2, 128), U32),
            pltpu.VMEM((NG, S // 2, 128), U32),
            pltpu.VMEM((NG, S // 2, 128), U32),
            pltpu.VMEM((NG, S // 2, 128), U32),
            pltpu.VMEM((NG, 128, S), BF16),
            pltpu.VMEM((7, 2, NP, S // 4, D), BF16),
            pltpu.VMEM((NP, 4, NE * SB, D), BF16),
            pltpu.VMEM((4, S - NE * SB, D), BF16),
            pltpu.VMEM((NS, 136, 128), F32),
            pltpu.VMEM((S + 32, 128), F32),
            pltpu.VMEM((1, S + 32, 128), F32),
            pltpu.VMEM((SH, 128), F32),
            pltpu.VMEM((2, S + 32, 128), F32),
            pltpu.VMEM((1, NCH, 6 * CH + 32, 128), F32),
            pltpu.VMEM((NCH, 2 * CH, 128), BF16),
            pltpu.VMEM((NG, SH, 128), BF16),
            pltpu.VMEM((NG // 2, SH, 128), BF16),
            pltpu.VMEM((NG // 2, SH, 128), BF16),
            pltpu.VMEM((NG, 8, 128), F32),
            pltpu.VMEM((2 * CH, CH), BF16),
            pltpu.VMEM((CH, CH), BF16),
            pltpu.VMEM((KS, M), BF16),
            pltpu.VMEM((NG, 128), BF16),
            pltpu.VMEM((NG, 128), BF16),
            pltpu.SemaphoreType.DMA((9 + NP // 2,)),
            pltpu.SemaphoreType.DMA((5,)),
            pltpu.SemaphoreType.DMA((3,)),
        ],
        compiler_params=pltpu.CompilerParams(vmem_limit_bytes=122 * 2**20),
    )(A_x.reshape(S, M), A_c_kv.reshape(S, DC), A_w_q, A_w_uk, A_w_uv,
      A_w_o.reshape(H * D, M), B_k.reshape(S, M), B_v.reshape(S, M), B_ssm_k,
      B_shift_k.T, B_ssm_D.reshape(NG, 128), gate_w.reshape(NG, 128), _FWD, _INV)
    return out.reshape(1, S, M)
```
